```python
import os as _os
_os.environ.setdefault("JAX_PLATFORMS", "cpu")
import jax
import jax.numpy as jnp

def _softmax(x, axis=-1):
    return jax.nn.softmax(x, axis=axis)
def _gelu(x):
    return jax.nn.gelu(x, approximate=True)
def _silu(x):
    return jax.nn.silu(x)
def _sigmoid(x):
    return jax.nn.sigmoid(x)
def _layernorm(x, axis=-1, eps=1e-5):
    m = jnp.mean(x, axis=axis, keepdims=True)
    v = jnp.var(x, axis=axis, keepdims=True)
    return (x - m) / jnp.sqrt(v + eps)
def _scatter_add(tgt, idx, src, axis=0):
    return tgt.at[idx].add(src)
def _segment_sum(src, seg, n):
    return jax.ops.segment_sum(src, seg, n)
class _Rng:
    def __init__(self, key):
        self._k = key
    def _next(self):
        self._k, sub = jax.random.split(self._k)
        return sub
    def normal(self, shape):
        return jax.random.normal(self._next(), shape, dtype=jnp.bfloat16)
    def randint(self, lo, hi, shape):
        return jax.random.randint(self._next(), shape, lo, hi, dtype=jnp.int32)
    def uniform(self, shape, lo=0.0, hi=1.0):
        return jax.random.uniform(self._next(), shape, jnp.bfloat16, lo, hi)
    def permutation(self, n):
        return jax.random.permutation(self._next(), n)


kernel_name = 'gated_mix__grouped_kv_mqa__glu_gated_reglu__prompt'

def setup_inputs():
    _rng = _Rng(jax.random.key(int.from_bytes(__import__("os").urandom(4), "little")))
    _w = (lambda a: (lambda t: t.astype(jnp.bfloat16) if jnp.issubdtype(t.dtype, jnp.floating) else t)(jnp.asarray(a)))
    def _A_setup():
        B, S, D, H = 1, 2048, 1024, 32
        Dh = D // H
        return {
            "x": _w((lambda *s: _rng.normal(s) * 0.05)(B, S, D)),
            "wq": _w((lambda *s: _rng.normal(s) * 0.2)(D, H * Dh)),
            "wk": _w((lambda *s: _rng.normal(s) * 0.2)(D, Dh)),
            "wv": _w((lambda *s: _rng.normal(s) * 0.05)(D, Dh)),
            "wo": _w((lambda *s: _rng.normal(s) * 0.05)(H * Dh, D)),
        }
    _A_in = _A_setup()

    def _B_setup():
        B, S, D, F = 1, 2048, 1024, 3584
        return {
            "x": _w((lambda *s: _rng.normal(s) * 0.05)(B, S, D)),
            "W_gate": _w((lambda *s: _rng.normal(s) * 0.8)(D, F) * (2.0 / D) ** 0.5),
            "W_up": _w((lambda *s: _rng.normal(s) * 0.8)(D, F) * (2.0 / D) ** 0.5),
            "W_down": _w((lambda *s: _rng.normal(s) * 0.8)(F, D) * (1.0 / F) ** 0.5),
        }
    _B_in = _B_setup()

    return {
        "A_x": _A_in["x"],
        "A_wq": _A_in["wq"],
        "A_wk": _A_in["wk"],
        "A_wv": _A_in["wv"],
        "A_wo": _A_in["wo"],
        "B_x": _B_in["x"],
        "B_W_gate": _B_in["W_gate"],
        "B_W_up": _B_in["W_up"],
        "B_W_down": _B_in["W_down"],
        "gate_w": _w((lambda *s: _rng.normal(s) * 0.05)(1024) * 16.0),
    }

def reference(A_x, A_wq, A_wk, A_wv, A_wo, B_x, B_W_gate, B_W_up, B_W_down, gate_w):
    def _A_ref(x, wq, wk, wv, wo):
        B, S, D = x.shape
        H = 32
        Dh = D // H
        q = (lambda x, *d: x.transpose(*d))((x @ wq).reshape(B, S, H, Dh), 0, 2, 1, 3)
        k = x @ wk
        v = x @ wv
        scores = jnp.einsum("bhqd,bkd->bhqk", q, k) * (Dh ** -0.5)
        p = _softmax(scores, axis=-1)
        o = jnp.einsum("bhqk,bkd->bhqd", p, v)
        return (lambda x, *d: x.transpose(*d))(o, 0, 2, 1, 3).reshape(B, S, H * Dh) @ wo

    def _B_ref(x, W_gate, W_up, W_down):
        gate = jnp.einsum("bsd,df->bsf", x, W_gate)
        up = jnp.einsum("bsd,df->bsf", x, W_up)
        gate = gate * (lambda x, dt: x.astype(dt))(gate > 0, gate.dtype)
        h = gate * up
        return jnp.einsum("bsf,fd->bsd", h, W_down)

    x = A_x
    g = _sigmoid((x * gate_w).sum(-1, keepdims=True))
    a = _A_ref(x, A_wq, A_wk, A_wv, A_wo)
    b = _B_ref(x, B_W_gate, B_W_up, B_W_down)
    return g * a + (1 - g) * b
```

```python
import functools
import math

import jax
import jax.numpy as jnp
import jax.experimental.pallas as pl
import jax.experimental.pallas.tpu as pltpu

H = 32
DH = 32
TQ = 512
KC = 256
FN = 128
OC = 512
SCOPES = 0

F32 = jnp.float32
BF16 = jnp.bfloat16
NT = (((1,), (1,)), ((), ()))


def _scope(name):
    import contextlib
    return jax.named_scope(name) if SCOPES else contextlib.nullcontext()


def _kernel(x_hbm, wq_hbm, wkt_hbm, wvt_hbm, wo_hbm, wg_hbm, wu_hbm, wd_hbm, gw_hbm,
            o_ref, x_ref, wq_ref, wkv_ref, wo_ref, wg_ref, wu_ref, wd_ref, gw_ref,
            k4_ref, vt_ref, s0_ref, s1_ref, on_ref, h_ref, g_ref,
            sem_x, sem_g, sem_u, sem_m):
    i = pl.program_id(0)
    S, D = x_ref.shape
    F = wg_ref.shape[1]
    nkc = S // KC
    NG = H // 4
    FH = TQ // 2
    FW = F // (NG // 2)
    nparts = FW // FN * FSPLIT
    XC = S // NXC

    def cp_x(c):
        rows = pl.ds(c * XC, XC)
        return pltpu.make_async_copy(x_hbm.at[rows, :], x_ref.at[rows, :], sem_x.at[c])

    def cp_cols(src, dst, sems, c):
        cols = pl.ds(pl.multiple_of(c * FW, 128), FW)
        return pltpu.make_async_copy(src.at[:, cols], dst.at[:, cols], sems.at[c])

    cp_wk = lambda: pltpu.make_async_copy(wkt_hbm, wkv_ref.at[pl.ds(0, DH), :], sem_m.at[0])
    cp_wv = lambda: pltpu.make_async_copy(wvt_hbm, wkv_ref.at[pl.ds(DH, DH), :], sem_m.at[1])
    cp_wq0 = lambda: pltpu.make_async_copy(
        wq_hbm.at[:, pl.ds(0, 128)], wq_ref.at[:, pl.ds(0, 128)], sem_m.at[2])
    cp_wq1 = lambda: pltpu.make_async_copy(
        wq_hbm.at[:, pl.ds(128, D - 128)], wq_ref.at[:, pl.ds(128, D - 128)], sem_m.at[3])
    cp_wo = lambda: pltpu.make_async_copy(wo_hbm, wo_ref, sem_m.at[4])
    cp_wd = lambda: pltpu.make_async_copy(wd_hbm, wd_ref, sem_m.at[5])
    cp_gw = lambda: pltpu.make_async_copy(gw_hbm, gw_ref, sem_m.at[6])

    @pl.when(i == 0)
    def _():
        with _scope("kvprep"):
            cp_wk().start()
            cp_wv().start()
            for c in range(NXC):
                cp_x(c).start()
            if EARLY:
                cp_wq0().start()
                cp_cols(wg_hbm, wg_ref, sem_g, 0).start()
                cp_cols(wu_hbm, wu_ref, sem_u, 0).start()
            cp_wk().wait()
            cp_wv().wait()
            for c in range(NXC):
                cp_x(c).wait()
                if c == 0 and not EARLY:
                    cp_wq0().start()
                    cp_cols(wg_hbm, wg_ref, sem_g, 0).start()
                    cp_cols(wu_hbm, wu_ref, sem_u, 0).start()
                if c == NXC - 1:
                    cp_wq1().start()
                    for cc in range(1, NG // 2):
                        cp_cols(wg_hbm, wg_ref, sem_g, cc).start()
                        cp_cols(wu_hbm, wu_ref, sem_u, cc).start()
                    cp_wo().start()
                    cp_wd().start()
                    cp_gw().start()
                rows = pl.ds(c * XC, XC)
                kvt = jax.lax.dot_general(wkv_ref[...], x_ref[rows, :], NT,
                                          preferred_element_type=F32)
                vt_ref[:, rows] = kvt[DH:].astype(BF16)
                kt = kvt[:DH]
                kk = jnp.concatenate([kt, kt, kt, kt], axis=0).T
                lane = jax.lax.broadcasted_iota(jnp.int32, kk.shape, 1)
                for j in range(4):
                    sel = jnp.logical_and(lane >= j * DH, lane < (j + 1) * DH)
                    k4_ref[j, rows, :] = jnp.where(sel, kk, 0.0).astype(BF16)
            cp_wq0().wait()

    row0 = pl.multiple_of(i * TQ, TQ)
    qscale = (DH ** -0.5) * math.log2(math.e)

    def group(g, carry):
        frow = pl.multiple_of((g % 2) * FH, FH)
        fcol0 = (g // 2) * FW

        @pl.when(jnp.logical_and(i == 0, g % 2 == 0))
        def _():
            cp_cols(wg_hbm, wg_ref, sem_g, g // 2).wait()
            cp_cols(wu_hbm, wu_ref, sem_u, g // 2).wait()

        @pl.when(jnp.logical_and(i == 0, g == 1))
        def _():
            cp_wq1().wait()

        def ffn_part(tt):
            t, r = tt // FSPLIT, tt % FSPLIT
            FR = FH // FSPLIT
            r0 = pl.multiple_of(frow + r * FR, FR)
            xh = x_ref[pl.ds(pl.multiple_of(row0 + r0, FR), FR), :]
            cols = pl.ds(pl.multiple_of(fcol0 + t * FN, 128), FN)
            gate = jnp.dot(xh, wg_ref[:, cols], preferred_element_type=F32)
            up = jnp.dot(xh, wu_ref[:, cols], preferred_element_type=F32)
            h_ref[pl.ds(r0, FR), cols] = (jnp.maximum(gate, 0.0) * up).astype(BF16)

        gcols = pl.ds(pl.multiple_of(g * 128, 128), 128)
        xt = x_ref[pl.ds(row0, TQ), :]
        qg = (jnp.dot(xt, wq_ref[:, gcols], preferred_element_type=F32) * qscale).T.astype(BF16)

        part_at = {}
        for t in range(nparts):
            part_at.setdefault(PART_SLOTS[t], []).append(t)

        def parts(slot):
            for t in part_at.get(slot, []):
                ffn_part(t)

        sbuf = (s0_ref, s1_ref)
        zoff = pl.multiple_of((i // 4096) * KB, KB)
        nsub = KC // KB

        outs = []
        m_prev = None
        parts(-1)
        for st in range(5):
            ja = st if st < 4 else None
            jb = st - 1 if st > 0 else None
            m8 = None
            l8 = None
            acc = None
            m8_hist = []
            for c in range(nkc):
                rows = pl.ds(c * KC, KC)
                if ja is not None:
                    s = jnp.dot(k4_ref[ja, rows, :], qg, preferred_element_type=F32)
                    sbuf[ja % 2][rows, :] = s
                    for r in range(KC // 8):
                        sr = s[r * 8:(r + 1) * 8, :]
                        m8 = sr if m8 is None else jnp.maximum(m8, sr)
                        if (r + 1) % (KB // 8) == 0:
                            m8_hist.append(m8)
                parts(st * nkc + c)
                if jb is not None:
                    for t in range(nsub):
                        k = c * nsub + t
                        sv = sbuf[jb % 2][pl.ds(zoff + k * KB, KB), :]
                        mu = mu0
                        if ja is not None and k - LAG >= 0:
                            mu = jnp.maximum(mu, jnp.minimum(mu, m8_hist[k - LAG]))
                        p = jnp.exp2(sv.reshape(KB // 8, 8, TQ) - mu[None]).reshape(KB, TQ)
                        for tt in range(KB // 128):
                            for r in reversed(range(16)):
                                r0 = tt * 128 + r * 8
                                pr = p[r0:r0 + 8, :]
                                l8 = pr if l8 is None else l8 + pr
                        pv = jnp.dot(vt_ref[:, pl.ds(k * KB, KB)], p.astype(BF16),
                                     preferred_element_type=F32)
                        acc = pv if acc is None else acc + pv
            if jb is not None:
                l = jnp.sum(l8, axis=0, keepdims=True)
                outs.append(acc / l)
            if ja is not None:
                mu0 = jnp.broadcast_to(jnp.max(m8, axis=0, keepdims=True), (8, TQ))
        units = range(5 * nkc)
        parts(len(units))
        og = jnp.concatenate(outs, axis=0).T
        on_ref[:, gcols] = og.astype(BF16)
        return carry

    with _scope("groups"):
        jax.lax.fori_loop(0, NG, group, 0)

    @pl.when(i == 0)
    def _():
        cp_wo().wait()
        cp_wd().wait()
        cp_gw().wait()

    with _scope("down"):
        xt = x_ref[pl.ds(row0, TQ), :]
        gw = gw_ref[...].astype(F32).reshape(1, D)
        z = jnp.sum(xt.astype(F32) * gw, axis=-1, keepdims=True)
        g_ref[...] = jnp.broadcast_to(jax.nn.sigmoid(z), g_ref.shape)

        def down_chunk(c, carry):
            cols = pl.ds(pl.multiple_of(c * OC, OC), OC)
            a = jnp.dot(on_ref[...], wo_ref[:, cols], preferred_element_type=F32)
            b = jnp.dot(h_ref[...], wd_ref[:, cols], preferred_element_type=F32)
            gt = jnp.concatenate([g_ref[...]] * (OC // 128), axis=1)
            o_ref[:, cols] = (gt * a + (1.0 - gt) * b).astype(o_ref.dtype)
            return carry
        jax.lax.fori_loop(0, D // OC, down_chunk, 0)


PART_SLOTS = (-1, 8, 16, 24, 32, 36, 40)
NXC = 4
EARLY = 0
FSPLIT = 1
LAG = 2
KB = 128


@jax.jit
def pallas_gated_mix__grouped_kv_mqa__glu_gated_reglu__prompt_kernel(
    A_x, A_wq, A_wk, A_wv, A_wo, B_x, B_W_gate, B_W_up, B_W_down, gate_w):
    B, S, D = A_x.shape
    F = B_W_gate.shape[1]
    x = A_x.reshape(S, D)

    out = pl.pallas_call(
        _kernel,
        grid=(S // TQ,),
        in_specs=[pl.BlockSpec(memory_space=pl.ANY)] * 9,
        out_specs=pl.BlockSpec((TQ, D), lambda i: (i, 0)),
        out_shape=jax.ShapeDtypeStruct((S, D), A_x.dtype),
        scratch_shapes=[
            pltpu.VMEM((S, D), BF16),
            pltpu.VMEM((D, D), BF16),
            pltpu.VMEM((2 * DH, D), BF16),
            pltpu.VMEM((D, D), BF16),
            pltpu.VMEM((D, F), BF16),
            pltpu.VMEM((D, F), BF16),
            pltpu.VMEM((F, D), BF16),
            pltpu.VMEM((D,), BF16),
            pltpu.VMEM((4, S, 128), BF16),
            pltpu.VMEM((DH, S), BF16),
            pltpu.VMEM((S, TQ), F32),
            pltpu.VMEM((S, TQ), F32),
            pltpu.VMEM((TQ, D), BF16),
            pltpu.VMEM((TQ, F), BF16),
            pltpu.VMEM((TQ, 128), F32),
            pltpu.SemaphoreType.DMA((NXC,)),
            pltpu.SemaphoreType.DMA((4,)),
            pltpu.SemaphoreType.DMA((4,)),
            pltpu.SemaphoreType.DMA((7,)),
        ],
        compiler_params=pltpu.CompilerParams(
            dimension_semantics=("arbitrary",),
            vmem_limit_bytes=100 * 1024 * 1024),
        name="gated_mix",
    )(x, A_wq, A_wk.T, A_wv.T, A_wo, B_W_gate, B_W_up, B_W_down, gate_w)
    return out.reshape(B, S, D)
```

```python
import contextlib
import math

import jax
import jax.numpy as jnp
import jax.experimental.pallas as pl
import jax.experimental.pallas.tpu as pltpu

H = 32
DH = 32
TQ = 512
KC = 256
KB = 128
NTK = 4
LAG = 6
LLAG = 4
GPI = 2
FU = 256
OR = 128
DPI = 2
NXC = 4
PADW = 128
PIECES = ((0, 256), (8, 256), (16, 256), (24, 256), (32, 256), (40, 256), (48, 256), (56, 256), (64, 128), (65, 128), (66, 128), (67, 128), (68, 128), (69, 128), (70, 128), (71, 128), (72, 256))
TIES = {256: (96, 128, 160, 192, 224, 256), 128: (48, 64, 80, 96, 112, 128)}
GTIES = (32, 64, 96, 128)
Q1_SLOT = 24
GATE_SLOT = 2
PEEL = 1
SCOPES = 0

F32 = jnp.float32
BF16 = jnp.bfloat16
NT = (((1,), (1,)), ((), ()))


def _scope(name):
    return jax.named_scope(name) if SCOPES else contextlib.nullcontext()


def _kernel(x_hbm, wq_hbm, wkt_hbm, wvt_hbm, wo_hbm, wg_hbm, wu_hbm, wd_hbm, gw_hbm,
            o_hbm, x_ref, wq_ref, wkv_ref, wo_ref, wgu_ref, wd_ref, gw_ref,
            k4_ref, vt_ref, s0_ref, s1_ref, on_ref, h_ref, g_ref, out_ref,
            sem_x, sem_q, sem_w, sem_m, sem_o):
    S, D = x_ref.shape
    F = wg_hbm.shape[1]
    nkc = S // KC
    nsub = KC // KB
    NQI = H // 4 // GPI
    NIT = (S // TQ) * NQI
    NH = 4 * GPI
    GR = S // NIT
    NRB = S // FU
    NWC = F // 256
    U0 = 2 * NRB
    UPI = ((F // 128) * NRB - U0) // NIT
    XC = S // NXC
    XH = XC // 2

    def copy(src, dst, sem):
        return pltpu.make_async_copy(src, dst, sem)

    def slab(ref, ct):
        return ref.at[:, pl.ds(ct * 128, 128)]

    def cp_xrows(r0, nr, sem):
        rows = pl.ds(r0, nr)
        return copy(x_hbm.at[rows, :], x_ref.at[rows, :], sem)

    def cp_x(c):
        return cp_xrows(pl.multiple_of(c * XC, XC), XC, sem_x.at[c])

    def cps_q(c):
        return [copy(slab(wq_hbm, c * GPI + k), wq_ref.at[c, k], sem_q.at[c]) for k in range(GPI)]

    def cps_w(c, ks, sem):
        return ([copy(slab(wg_hbm, 2 * c + k), wgu_ref.at[c, k], sem) for k in ks]
                + [copy(slab(wu_hbm, 2 * c + k), wgu_ref.at[c, 2 + k], sem) for k in ks])

    def start(cps):
        for cp in cps:
            cp.start()

    def wait(cps):
        for cp in cps:
            cp.wait()

    cps_od = [copy(wo_hbm, wo_ref.at[:, pl.ds(0, D)], sem_m.at[2]),
              copy(wd_hbm, wd_ref.at[:, pl.ds(0, D)], sem_m.at[2])]

    def kv_rows(rows, xc):
        kvt = jax.lax.dot_general(wkv_ref[...], xc, NT, preferred_element_type=F32)
        vt_ref[:, rows] = kvt[DH:].astype(BF16)
        kt = kvt[:DH]
        kk = jnp.concatenate([kt, kt, kt, kt], axis=0).T
        lane = jax.lax.broadcasted_iota(jnp.int32, kk.shape, 1)
        for j in range(4):
            sel = jnp.logical_and(lane >= j * DH, lane < (j + 1) * DH)
            k4_ref[j, rows, :] = jnp.where(sel, kk, 0.0).astype(BF16)

    def ffn_rows(rows, xc, ks):
        wg0 = jnp.concatenate([wgu_ref[0, k] for k in ks], axis=1)
        wu0 = jnp.concatenate([wgu_ref[0, 2 + k] for k in ks], axis=1)
        gate = jnp.dot(xc, wg0, preferred_element_type=F32)
        up = jnp.dot(xc, wu0, preferred_element_type=F32)
        hh = (jnp.maximum(gate, 0.0) * up).astype(BF16)
        for i, k in enumerate(ks):
            h_ref[k, rows, :] = hh[:, i * 128:(i + 1) * 128]

    with _scope("kvprep"):
        small = [copy(wkt_hbm, wkv_ref.at[pl.ds(0, DH), :], sem_m.at[0]),
                 copy(wvt_hbm, wkv_ref.at[pl.ds(DH, DH), :], sem_m.at[0]),
                 copy(gw_hbm, gw_ref, sem_m.at[0])]
        if PEEL:
            batch_a = [cp_xrows(0, XH, sem_m.at[3])] + cps_w(0, [0], sem_m.at[3])
            batch_b = [cp_xrows(XH, XH, sem_m.at[1])] + cps_w(0, [1], sem_m.at[1])
            start(small)
            start(batch_a)
            wait(small)
            start(batch_b)
            wait(batch_a)
            with _scope("p1"):
                rows = pl.ds(0, XH)
                xc = x_ref[rows, :]
                ffn_rows(rows, xc, [0])
                kv_rows(rows, xc)
            wait(batch_b)
            cp_x(1).start()
            with _scope("p2"):
                ffn_rows(rows, x_ref[rows, :], [1])
                rows = pl.ds(XH, XH)
                xc = x_ref[rows, :]
                kv_rows(rows, xc)
                ffn_rows(rows, xc, [0, 1])
        else:
            batch_a = small + cps_w(0, [0, 1], sem_m.at[0])
            start(batch_a)
            cp_x(0).start()
            wait(batch_a)

        def prep(c, carry):
            cp_x(c).wait()

            @pl.when(c + 1 < NXC)
            def _():
                cp_x(c + 1).start()

            @pl.when(c == NXC - 2)
            def _():
                start(cps_q(0) + cps_w(1, [0, 1], sem_w.at[1]))

            rows = pl.ds(pl.multiple_of(c * XC, XC), XC)
            xc = x_ref[rows, :]
            kv_rows(rows, xc)
            ffn_rows(rows, xc, [0, 1])
            return carry
        jax.lax.fori_loop(PEEL, NXC, prep, 0)
        for c in range(2, NWC):
            if c - 1 < NQI:
                start(cps_q(c - 1))
            start(cps_w(c, [0, 1], sem_w.at[c]))
        start(cps_od)

    qscale = (DH ** -0.5) * math.log2(math.e)

    def body(n, carry):
        with _scope('iter'):
            return body_(n, carry)

    def body_(n, carry):
        @pl.when(n < NQI)
        def _():
            copy(wq_ref.at[n], wq_ref.at[n], sem_q.at[n]).wait()

        @pl.when(n + 1 < NWC)
        def _():
            copy(wgu_ref.at[n + 1], wgu_ref.at[n + 1], sem_w.at[n + 1]).wait()

        t = jnp.bitwise_and(n, NQI - 1)
        row0 = pl.multiple_of(jnp.right_shift(n, NQI.bit_length() - 1) * TQ, TQ)

        clock = []
        gclock = []

        def tick(v, dst=clock):
            ninf = jnp.minimum(v, -jnp.inf)
            dst.append(jnp.concatenate([ninf] * (TQ // 128), axis=1))

        def ffn_piece(j, r0, nr):
            u = U0 + n * UPI + j
            ct = jnp.right_shift(u, NRB.bit_length() - 1)
            rb = jnp.bitwise_and(u, NRB - 1)
            wc = jnp.right_shift(ct, 1)
            wk = jnp.bitwise_and(ct, 1)
            rows = pl.ds(pl.multiple_of(rb * FU + r0, 128), nr)
            xh = x_ref[rows, :]
            gate = jnp.dot(xh, wgu_ref[wc, wk], preferred_element_type=F32)
            up = jnp.dot(xh, wgu_ref[wc, 2 + wk], preferred_element_type=F32)
            hh = jnp.maximum(gate, 0.0) * up
            h_ref[ct, rows, :] = hh.astype(BF16)
            for ra in TIES[nr]:
                tick(hh[ra - 8:ra])
            if nr == 128:
                gclock.clear()
                for ra in GTIES:
                    tick(gate[ra - 8:ra], gclock)

        def qproj(gl):
            xt = x_ref[pl.ds(row0, TQ), :]
            q = jnp.dot(xt, wq_ref[t, gl], preferred_element_type=F32)
            return (q * qscale).T.astype(BF16)

        def gate_rows():
            rows = pl.ds(pl.multiple_of(n * GR, GR), GR)
            xg = x_ref[rows, :].astype(F32)
            gw = gw_ref[...].astype(F32).reshape(1, D)
            z = jnp.sum(xg * gw, axis=-1, keepdims=True)
            g_ref[rows, :] = jnp.broadcast_to(jax.nn.sigmoid(z), (GR, 128))

        sched = {}
        j, r0 = 0, 0
        for slot, nr in PIECES:
            sched.setdefault(slot, []).append((j, r0, nr))
            r0 += nr
            if r0 == FU:
                j, r0 = j + 1, 0
        assert j == UPI and r0 == 0

        qg = [qproj(0)]

        def fill(slot):
            if slot == Q1_SLOT:
                for gl in range(1, GPI):
                    qg.append(qproj(gl))
            if slot == GATE_SLOT:
                gate_rows()
            for pc in sched.get(slot, []):
                ffn_piece(*pc)

        sbuf = (s0_ref, s1_ref)
        RB = KB // NTK

        outs = []
        for st in range(NH + 1):
            ja = st if st < NH else None
            jb = st - 1 if st > 0 else None
            m8 = None
            l8 = None
            acc = None
            for c in range(nkc):
                rows = pl.ds(c * KC, KC)
                base0 = len(clock)
                fill(st * nkc + c)
                base = len(clock)
                if ja is not None:
                    s = jnp.dot(k4_ref[ja % 4, rows, :], qg[ja // 4], preferred_element_type=F32)
                    sbuf[ja % 2][rows, :] = s
                    for r in range(KC // 8):
                        sr = s[r * 8:(r + 1) * 8, :]
                        m8 = sr if m8 is None else jnp.maximum(m8, sr)
                        if (r + 1) % (RB // 8) == 0:
                            tick(m8[:, :128])
                if jb is not None:
                    for tt in range(nsub):
                        k = c * nsub + tt
                        ps = []
                        for u in range(NTK):
                            lo = KB - (u + 1) * RB
                            sv = sbuf[jb % 2][pl.ds(k * KB + lo, RB), :]
                            gi = tt * NTK + u
                            nearly = nsub * NTK - len(GTIES)
                            if ja is not None:
                                clk = clock[base - LAG + gi]
                            elif gi < nearly:
                                clk = clock[min(base0 - LLAG + gi, base0 - 1)]
                            else:
                                clk = gclock[gi - nearly]
                            mu = jnp.maximum(mu0, clk)
                            pu = jnp.exp2(sv.reshape(RB // 8, 8, TQ) - mu[None]).reshape(RB, TQ)
                            for r in reversed(range(RB // 8)):
                                pr = pu[r * 8:(r + 1) * 8, :]
                                l8 = pr if l8 is None else l8 + pr
                            ps.insert(0, pu)
                        p = jnp.concatenate(ps, axis=0).astype(BF16)
                        pv = jnp.dot(vt_ref[:, pl.ds(k * KB, KB)], p,
                                     preferred_element_type=F32)
                        acc = pv if acc is None else acc + pv
                        tick(pv[DH - 8:, :128])
            if jb is not None:
                l = jnp.sum(l8, axis=0, keepdims=True)
                outs.append(acc / l)
                if jb == NH - 1:
                    fill((NH + 1) * nkc)
                if jb % 4 == 3:
                    og = jnp.concatenate(outs, axis=0).T
                    on_ref[t * GPI + jb // 4, pl.ds(row0, TQ), :] = og.astype(BF16)
                    outs = []
            if ja is not None:
                mu0 = jnp.broadcast_to(jnp.max(m8, axis=0, keepdims=True), (8, TQ))
        return carry

    with _scope("groups"):
        jax.lax.fori_loop(0, NIT, body, 0)

    wait(cps_od)

    nob = S // OR

    def cp_out(c):
        rows = pl.ds(pl.multiple_of(c * OR, OR), OR)
        return copy(out_ref.at[rows, :], o_hbm.at[rows, :], sem_o.at[0])

    with _scope("down"):
        def down_block(c):
            rows = pl.ds(pl.multiple_of(c * OR, OR), OR)
            on = jnp.concatenate([on_ref[k, rows, :] for k in range(D // 128)], axis=1)
            hv = jnp.concatenate([h_ref[k, rows, :] for k in range(F // 128)], axis=1)
            a = jnp.dot(on, wo_ref[:, :D], preferred_element_type=F32)
            b = jnp.dot(hv, wd_ref[:, :D], preferred_element_type=F32)
            gt = jnp.concatenate([g_ref[rows, :]] * (D // 128), axis=1)
            out_ref[rows, :] = (gt * a + (1.0 - gt) * b).astype(out_ref.dtype)
            cp_out(c).start()

        def down_chunk(c, carry):
            for k in range(DPI):
                down_block(c * DPI + k)
            return carry
        jax.lax.fori_loop(0, nob // DPI, down_chunk, 0)

    copy(out_ref, o_hbm, sem_o.at[0]).wait()


@jax.jit
def pallas_gated_mix__grouped_kv_mqa__glu_gated_reglu__prompt_kernel(
    A_x, A_wq, A_wk, A_wv, A_wo, B_x, B_W_gate, B_W_up, B_W_down, gate_w):
    B, S, D = A_x.shape
    F = B_W_gate.shape[1]
    x = A_x.reshape(S, D)
    nqi = H // 4 // GPI

    out = pl.pallas_call(
        _kernel,
        in_specs=[pl.BlockSpec(memory_space=pl.ANY)] * 9,
        out_specs=pl.BlockSpec(memory_space=pl.ANY),
        out_shape=jax.ShapeDtypeStruct((S, D), A_x.dtype),
        scratch_shapes=[
            pltpu.VMEM((S, D), BF16),
            pltpu.VMEM((nqi, GPI, D, 128), BF16),
            pltpu.VMEM((2 * DH, D), BF16),
            pltpu.VMEM((D, D + PADW), BF16),
            pltpu.VMEM((F // 256, 4, D, 128), BF16),
            pltpu.VMEM((F, D + PADW), BF16),
            pltpu.VMEM((D,), BF16),
            pltpu.VMEM((4, S, 128), BF16),
            pltpu.VMEM((DH, S), BF16),
            pltpu.VMEM((S, TQ), F32),
            pltpu.VMEM((S, TQ), F32),
            pltpu.VMEM((D // 128, S, 128), BF16),
            pltpu.VMEM((F // 128, S, 128), BF16),
            pltpu.VMEM((S, 128), F32),
            pltpu.VMEM((S, D), BF16),
            pltpu.SemaphoreType.DMA((NXC,)),
            pltpu.SemaphoreType.DMA((nqi,)),
            pltpu.SemaphoreType.DMA((F // 256,)),
            pltpu.SemaphoreType.DMA((4,)),
            pltpu.SemaphoreType.DMA((1,)),
        ],
        compiler_params=pltpu.CompilerParams(
            vmem_limit_bytes=100 * 1024 * 1024,
            disable_bounds_checks=True,
            disable_semaphore_checks=True),
        name="gated_mix",
    )(x, A_wq, A_wk.T, A_wv.T, A_wo, B_W_gate, B_W_up, B_W_down, gate_w)
    return out.reshape(B, S, D)
```

```python
import math

import jax
import jax.numpy as jnp
import jax.experimental.pallas as pl
import jax.experimental.pallas.tpu as pltpu

H = 32
DH = 32
TQ = 512
KC = 256
KB = 128
NTK = 4
LAG = 6
GPI = 2
FU = 256
NXC = 4
PADW = 128
KV = 192
VR = 2
GU_SLOTS = (0, 4, 8, 12, 16, 20, 24, 28, 32, 40, 44, 48, 56)
DN_SLOTS = (2, 6, 10, 14, 18, 22, 26, 30, (64, 65), (66, 67), (68, 69), (70, 71), 72)
OP_SLOTS = (52, 72)
Q1_SLOT = 8
TIES = (8, 56, 104, 144, 192, 240)
STIES = (8, 8, 8, 32, 64, 96, 128, 160)

F32 = jnp.float32
BF16 = jnp.bfloat16
NT = (((1,), (1,)), ((), ()))


def _kernel(x_hbm, wq_hbm, wkt_hbm, wvt_hbm, wo_hbm, wg_hbm, wu_hbm, wd_hbm, gw_hbm,
            o_hbm, x_ref, wq_ref, wkv_ref, wo_ref, wgu_ref, wd_ref, gw_ref,
            k4_ref, vt_ref, s0_ref, s1_ref, g_ref, acc_ref, out_ref,
            kb_ref, qf_ref, sv_ref,
            sem_x, sem_q, sem_o, sem_w, sem_d, sem_m, sem_out):
    S, D = x_ref.shape
    nkc = S // KC
    nsub = KC // KB
    NQI = H // 4 // GPI
    NIT = (S // TQ) * NQI
    NH = 4 * GPI
    XC = S // NXC
    XH = XC // 2
    FR = TQ // NQI
    NCT = TQ // 128
    NVP = KV // 8 // VR
    RB = KB // NTK
    qscale = (DH ** -0.5) * math.log2(math.e)

    def copy(src, dst, sem):
        return pltpu.make_async_copy(src, dst, sem)

    def start(cps):
        for cp in cps:
            cp.start()

    def wait(cps):
        for cp in cps:
            cp.wait()

    def cp_x(c):
        rows = pl.ds(pl.multiple_of(c * XC, XC), XC)
        return copy(x_hbm.at[rows, :], x_ref.at[rows, :], sem_x.at[c])

    def cp_xh(k, sem):
        rows = pl.ds(k * XH, XH)
        return copy(x_hbm.at[rows, :], x_ref.at[rows, :], sem)

    def cps_q(t):
        return [copy(wq_hbm.at[:, pl.ds((t * GPI + k) * 128, 128)], wq_ref.at[t, k], sem_q.at[t])
                for k in range(GPI)]

    def cp_rows(src, dst, r0, nr, sem):
        return copy(src.at[pl.ds(r0, nr), :], dst.at[pl.ds(r0, nr), pl.ds(0, D)], sem)

    def cp_wo(t):
        r0 = t * (GPI * 128)
        if not isinstance(t, int):
            r0 = pl.multiple_of(r0, GPI * 128)
        return cp_rows(wo_hbm, wo_ref, r0, GPI * 128, sem_o.at[t])

    def cps_gu(s0, ns, sem):
        cps = []
        for s in range(s0, s0 + ns):
            cols = pl.ds(s * 128, 128)
            cps.append(copy(wg_hbm.at[:, cols], wgu_ref.at[s, 0], sem))
            cps.append(copy(wu_hbm.at[:, cols], wgu_ref.at[s, 1], sem))
        return cps

    def cp_out(b):
        rows = pl.ds(pl.multiple_of(b * FR, FR), FR)
        return copy(out_ref.at[rows, :], o_hbm.at[rows, :], sem_out.at[0])

    def chunk(t):
        return 2 + 13 * (t // 2) + 7 * (t % 2), 7 - t % 2

    def kv_rows(rows, xc):
        kvt = jax.lax.dot_general(wkv_ref[...], xc, NT, preferred_element_type=F32)
        vt_ref[:, rows] = kvt[DH:].astype(BF16)
        kt = kvt[:DH]
        kk = jnp.concatenate([kt, kt, kt, kt], axis=0).T
        lane = jax.lax.broadcasted_iota(jnp.int32, kk.shape, 1)
        for j in range(4):
            sel = jnp.logical_and(lane >= j * DH, lane < (j + 1) * DH)
            k4_ref[j, rows, :] = jnp.where(sel, kk, 0.0).astype(BF16)

    def gate_rows(rows, xc):
        gw = gw_ref[...].astype(F32).reshape(1, D)
        z = jnp.sum(xc.astype(F32) * gw, axis=-1, keepdims=True)
        g = jnp.broadcast_to(jax.nn.sigmoid(z), (xc.shape[0], 128))
        g_ref[rows, :] = g
        return 1.0 - g

    def hidden(xc, om, ks):
        wg0 = jnp.concatenate([wgu_ref[k, 0] for k in ks], axis=1)
        wu0 = jnp.concatenate([wgu_ref[k, 1] for k in ks], axis=1)
        gate = jnp.dot(xc, wg0, preferred_element_type=F32)
        up = jnp.dot(xc, wu0, preferred_element_type=F32)
        om = jnp.concatenate([om] * len(ks), axis=1)
        return (jnp.maximum(gate, 0.0) * up * om).astype(BF16)

    def init_acc(rows, hh):
        acc_ref[rows, :] = jnp.dot(hh, wd_ref[:256, :D], preferred_element_type=F32)

    small = [copy(wkt_hbm, wkv_ref.at[pl.ds(0, DH), :], sem_m.at[0]),
             copy(wvt_hbm, wkv_ref.at[pl.ds(DH, DH), :], sem_m.at[0]),
             copy(gw_hbm, gw_ref, sem_m.at[0])]
    batch_a = [cp_xh(0, sem_m.at[1])] + cps_gu(0, 1, sem_m.at[1])
    batch_b = [cp_xh(1, sem_m.at[2])] + cps_gu(1, 1, sem_m.at[2])
    cp_wd0 = cp_rows(wd_hbm, wd_ref, 0, 256, sem_m.at[0])
    s0, ns = chunk(0)
    gu0 = cps_gu(s0, ns, sem_w.at[0])
    early = [gu0[:3], gu0[3:10], gu0[10:] + cps_q(0),
             [cp_rows(wd_hbm, wd_ref, s0 * 128, ns * 128, sem_d.at[0]), cp_wo(0)]]
    start(small)
    start(batch_a)
    wait(small)
    start(batch_b)
    wait(batch_a)

    rows0 = pl.ds(0, XH)
    xc = x_ref[rows0, :]
    om0 = gate_rows(rows0, xc)
    h0 = hidden(xc, om0, [0])
    kv_rows(rows0, xc)

    wait(batch_b)
    cp_wd0.start()
    cp_x(1).start()

    kr = k4_ref[0, :KV, :].astype(F32)
    for d in range(DH):
        kb_ref[d] = jnp.broadcast_to(kr[:, d:d + 1], (KV, 128))
    h1 = hidden(x_ref[rows0, :], om0, [1])
    rows1 = pl.ds(XH, XH)
    xc = x_ref[rows1, :]
    kv_rows(rows1, xc)
    h2 = hidden(xc, gate_rows(rows1, xc), [0, 1])

    cp_wd0.wait()
    start(early[0])
    init_acc(pl.ds(0, XC), jnp.concatenate([jnp.concatenate([h0, h1], axis=1), h2], axis=0))

    def prep(c, carry):
        cp_x(c).wait()

        @pl.when(c + 1 < NXC)
        def _():
            cp_x(c + 1).start()

        for k in range(1, NXC):
            @pl.when(c == k)
            def _():
                start(early[k])

        rows = pl.ds(pl.multiple_of(c * XC, XC), XC)
        xr = x_ref[rows, :]
        kv_rows(rows, xr)
        init_acc(rows, hidden(xr, gate_rows(rows, xr), [0, 1]))
        return carry

    jax.lax.fori_loop(1, NXC, prep, 0)
    for t in range(1, NQI):
        s0, ns = chunk(t)
        start(cps_q(t) + cps_gu(s0, ns, sem_w.at[t])
              + [cp_rows(wd_hbm, wd_ref, s0 * 128, ns * 128, sem_d.at[t]), cp_wo(t)])

    def body(n, carry):
        t = jnp.bitwise_and(n, NQI - 1)
        odd = jnp.bitwise_and(n, 1)
        sbase = 2 + 13 * jnp.right_shift(t, 1) + 7 * odd
        sextra = 8 + 13 * jnp.right_shift(t, 1)

        @pl.when(n < NQI)
        def _():
            copy(wq_ref.at[n], wq_ref.at[n], sem_q.at[n]).wait()
            cp_wo(n).wait()

        for par in range(2):
            @pl.when(jnp.logical_and(n < NQI, odd == par))
            def _():
                ns = 7 - par
                blk = wgu_ref.at[pl.ds(sbase, ns)]
                copy(blk, blk, sem_w.at[n]).wait()
                cp_rows(wd_hbm, wd_ref, pl.multiple_of(sbase * 128, 128), ns * 128,
                        sem_d.at[n]).wait()

        row0 = pl.multiple_of(jnp.right_shift(n, NQI.bit_length() - 1) * TQ, TQ)
        fb = jnp.where(n >= NQI, n - NQI, n)
        nfin = [0]

        @pl.when(n > NQI)
        def _():
            cp_out(n - NQI - 1).start()

        def finalize_piece():
            k = nfin[0]
            nfin[0] += 1
            if k < FR // 8:
                rows = pl.ds(pl.multiple_of(fb * FR + k * 8, 8), 8)
                out_ref[rows, :] = acc_ref[rows, :].astype(out_ref.dtype)

        clock = []
        sclock = []
        vchain = [None]
        rot = [0]

        def tick(v, dst=clock):
            dst.append(jnp.minimum(v, -jnp.inf))

        def filler_ticks(res):
            for ra in TIES:
                tick(res[ra - 8:ra])
            sclock.clear()
            for ra in STIES:
                tick(res[ra - 8:ra], sclock)

        def unit(j):
            if j < 12:
                return sbase + j // 2, row0 + (j % 2) * FU
            return sextra, row0 + odd * FU

        hs = {}

        def gate_up(j):
            s, r0 = unit(j)
            rows = pl.ds(pl.multiple_of(r0, FU), FU)
            xh = x_ref[rows, :]
            gate = jnp.dot(xh, wgu_ref[s, 0], preferred_element_type=F32)
            up = jnp.dot(xh, wgu_ref[s, 1], preferred_element_type=F32)
            hh = jnp.maximum(gate, 0.0) * up
            filler_ticks(hh)
            hs[j] = (hh * (1.0 - g_ref[rows, :])).astype(BF16)

        def down(j, half):
            s, r0 = unit(j)
            lo, nr = (0, FU) if half is None else (half * (FU // 2), FU // 2)
            rows = pl.ds(pl.multiple_of(r0 + lo, nr), nr)
            w = wd_ref[pl.ds(pl.multiple_of(s * 128, 128), 128), :D]
            res = jnp.dot(hs[j][lo:lo + nr], w, preferred_element_type=F32)
            finalize_piece()
            acc_ref[rows, :] += res
            if half is None:
                filler_ticks(res[:, D - 128:])
            else:
                for c0 in (0, D - 128):
                    for ra in range(32, nr + 1, 32):
                        tick(res[ra - 8:ra, c0:c0 + 128])

        ogs = {}

        def out_proj(gl):
            rows = pl.ds(row0, TQ)
            w = wo_ref[pl.ds(pl.multiple_of((t * GPI + gl) * 128, 128), 128), :D]
            res = jnp.dot(ogs[gl], w, preferred_element_type=F32)
            finalize_piece()
            acc_ref[rows, :] += res
            filler_ticks(res[TQ - 256:, D - 128:])

        def qproj(gl):
            xt = x_ref[pl.ds(row0, TQ), :]
            q = jnp.dot(xt, wq_ref[t, gl], preferred_element_type=F32)
            qt = (q * qscale).T.astype(BF16)
            qtf = qt.astype(F32)
            for r in range(128):
                qf_ref[gl, r] = jnp.broadcast_to(qtf[r:r + 1, :], (8, TQ))
            return qt

        qg = [qproj(0)]
        mv = {}

        def vpu_part(j, vp):
            vrows = pl.ds(vp * VR * 8, VR * 8)
            gate_v = vchain[0]
            sacc = None
            for d in range(DH):
                kb = kb_ref[d, vrows, :].reshape(VR, 8, 128)
                if gate_v is not None:
                    kb = jnp.maximum(kb, gate_v[None])
                kb = jnp.concatenate([kb] * NCT, axis=2)
                prod = kb * qf_ref[j // 4, (j % 4) * DH + d][None]
                sacc = prod if sacc is None else sacc + prod
                ix = rot[0] % (VR * NCT)
                rot[0] += 1
                gate_v = jnp.minimum(
                    sacc[ix // NCT, :, (ix % NCT) * 128:(ix % NCT + 1) * 128], -jnp.inf)
            sv_ref[j, vrows, :] = sacc.reshape(VR * 8, TQ)
            for r in range(VR):
                mv[j] = sacc[r] if j not in mv else jnp.maximum(mv[j], sacc[r])
            for cc in range(NCT):
                gate_v = jnp.minimum(mv[j][:, cc * 128:(cc + 1) * 128], gate_v)
            vchain[0] = gate_v

        sched = {}
        for j, slot in enumerate(GU_SLOTS):
            sched.setdefault(slot, []).append((gate_up, (j,)))
        for j, slot in enumerate(DN_SLOTS):
            if isinstance(slot, tuple):
                for half in range(2):
                    sched.setdefault(slot[half], []).append((down, (j, half)))
            else:
                sched.setdefault(slot, []).append((down, (j, None)))
        for gl, slot in enumerate(OP_SLOTS):
            sched.setdefault(slot, []).append((out_proj, (gl,)))

        def fill(slot):
            if slot == Q1_SLOT:
                qg.append(qproj(1))
            for fn, a in sched.get(slot, []):
                fn(*a)
            for j in range(NH):
                if slot == max(j * nkc - 7, 0 if j < 4 else Q1_SLOT):
                    for vp in range(NVP):
                        vpu_part(j, vp)

        sbuf = (s0_ref, s1_ref)
        outs = []
        for st in range(NH + 1):
            ja = st if st < NH else None
            jb = st - 1 if st > 0 else None
            m8 = None
            l8 = None
            acc = None
            for c in range(nkc):
                base = len(clock)
                fill(st * nkc + c)
                if ja is not None:
                    base = len(clock)
                    lo_k = KV if c == 0 else c * KC
                    nk = (c + 1) * KC - lo_k
                    arows = pl.ds(lo_k, nk)
                    s = jnp.dot(k4_ref[ja % 4, arows, :], qg[ja // 4], preferred_element_type=F32)
                    sbuf[ja % 2][arows, :] = s
                    for r in range(nk // 8):
                        sr = s[r * 8:(r + 1) * 8, :]
                        m8 = sr if m8 is None else jnp.maximum(m8, sr)
                        if (r + 1) % (RB // 8) == 0:
                            tc = ((r + 1) // (RB // 8)) % NCT
                            tick(m8[:, tc * 128:(tc + 1) * 128])
                if jb is not None:
                    for tt in range(nsub):
                        k = c * nsub + tt
                        ps = []
                        for u in range(NTK):
                            lo = k * KB + KB - (u + 1) * RB
                            if lo < KV:
                                sv = sv_ref[jb, pl.ds(lo, RB), :]
                            else:
                                sv = sbuf[jb % 2][pl.ds(lo, RB), :]
                            gi = tt * NTK + u
                            if ja is not None and c == 0:
                                clk = sclock[gi]
                            else:
                                clk = clock[base - LAG + gi]
                            mu = jnp.maximum(mu0, jnp.concatenate([clk] * NCT, axis=1))
                            pu = jnp.exp2(sv.reshape(RB // 8, 8, TQ) - mu[None]).reshape(RB, TQ)
                            for r in reversed(range(RB // 8)):
                                pr = pu[r * 8:(r + 1) * 8, :]
                                l8 = pr if l8 is None else l8 + pr
                            ps.insert(0, pu)
                        p = jnp.concatenate(ps, axis=0).astype(BF16)
                        pv = jnp.dot(vt_ref[:, pl.ds(k * KB, KB)], p,
                                     preferred_element_type=F32)
                        acc = pv if acc is None else acc + pv
                        tick(pv[DH - 8:, :128])
            if jb is not None:
                l = jnp.sum(l8, axis=0, keepdims=True)
                outs.append(acc / l)
                if jb % 4 == 3:
                    og = jnp.concatenate(outs, axis=0).T
                    ogs[jb // 4] = (og * g_ref[pl.ds(row0, TQ), :]).astype(BF16)
                    outs = []
                if jb == NH - 1:
                    fill((NH + 1) * nkc)
            if ja is not None:
                m8 = jnp.maximum(m8, mv[ja])
                mu0 = jnp.broadcast_to(jnp.max(m8, axis=0, keepdims=True), (8, TQ))
        return carry

    jax.lax.fori_loop(0, NIT, body, 0)

    cp_out(NIT - NQI - 1).start()
    for b in range(NIT - NQI, NIT):
        rows = pl.ds(b * FR, FR)
        out_ref[rows, :] = acc_ref[rows, :].astype(out_ref.dtype)
        cp_out(b).start()
    copy(out_ref, o_hbm, sem_out.at[0]).wait()


@jax.jit
def pallas_gated_mix__grouped_kv_mqa__glu_gated_reglu__prompt_kernel(
    A_x: jax.Array,
    A_wq: jax.Array,
    A_wk: jax.Array,
    A_wv: jax.Array,
    A_wo: jax.Array,
    B_x: jax.Array,
    B_W_gate: jax.Array,
    B_W_up: jax.Array,
    B_W_down: jax.Array,
    gate_w: jax.Array,
):
    B, S, D = A_x.shape
    F = B_W_gate.shape[1]
    assert (B, S, D, F) == (1, 2048, 1024, 3584)
    x = A_x.reshape(S, D)
    nqi = H // 4 // GPI

    out = pl.pallas_call(
        _kernel,
        in_specs=[pl.BlockSpec(memory_space=pl.ANY)] * 9,
        out_specs=pl.BlockSpec(memory_space=pl.ANY),
        out_shape=jax.ShapeDtypeStruct((S, D), A_x.dtype),
        scratch_shapes=[
            pltpu.VMEM((S, D), BF16),
            pltpu.VMEM((nqi, GPI, D, 128), BF16),
            pltpu.VMEM((2 * DH, D), BF16),
            pltpu.VMEM((D, D + PADW), BF16),
            pltpu.VMEM((F // 128, 2, D, 128), BF16),
            pltpu.VMEM((F, D + PADW), BF16),
            pltpu.VMEM((D,), BF16),
            pltpu.VMEM((4, S, 128), BF16),
            pltpu.VMEM((DH, S), BF16),
            pltpu.VMEM((S, TQ), F32),
            pltpu.VMEM((S, TQ), F32),
            pltpu.VMEM((S, 128), F32),
            pltpu.VMEM((S, D), F32),
            pltpu.VMEM((S, D), BF16),
            pltpu.VMEM((DH, KV, 128), F32),
            pltpu.VMEM((GPI, 128, 8, TQ), F32),
            pltpu.VMEM((4 * GPI, KV, TQ), F32),
            pltpu.SemaphoreType.DMA((NXC,)),
            pltpu.SemaphoreType.DMA((nqi,)),
            pltpu.SemaphoreType.DMA((nqi,)),
            pltpu.SemaphoreType.DMA((nqi,)),
            pltpu.SemaphoreType.DMA((nqi,)),
            pltpu.SemaphoreType.DMA((3,)),
            pltpu.SemaphoreType.DMA((1,)),
        ],
        compiler_params=pltpu.CompilerParams(
            vmem_limit_bytes=110 * 1024 * 1024,
            disable_bounds_checks=True,
            disable_semaphore_checks=True),
        name="gated_mix",
    )(x, A_wq, A_wk.T, A_wv.T, A_wo, B_W_gate, B_W_up, B_W_down, gate_w)
    return out.reshape(B, S, D)
```

```python
import math

import jax
import jax.numpy as jnp
import jax.experimental.pallas as pl
import jax.experimental.pallas.tpu as pltpu

H = 32
DH = 32
TQ = 512
KC = 256
KB = 128
NTK = 4
LAGS = (
    (5, 6, 5, 5, 5, 5, 5, 5),
    (5, 6, 5, 5, 5, 5, 5, 5),
    (5, 6, 5, 5, 6, 5, 5, 5),
    (5, 6, 5, 5, 5, 6, 6, 6),
    (5, 6, 5, 5, 5, 5, 5, 5),
    (6, 7, 7, 6, 6, 6, 6, 7),
    (5, 6, 5, 5, 5, 5, 5, 5),
    (5, 6, 7, 5, 5, 5, 6, 5),
    (5, 5, 5, 5, 5, 5, 5, 6),
)
GPI = 2
FU = 256
NXC = 4
APH = 2
PADW = 128
KVS = (256, 208, 256, 224, 256, 224, 256, 320)
KV = max(max(KVS), 272)
ONL = (7,)
VR = 2
LB = 2
GU_SLOTS = (1, 4, 8, 10, 16, 18, 23, 24, 32, 40, 42, 48, 56)
DN_SLOTS = (4, 5, 10, 21, 19, 23, 29, 38, (64, 65), (66, 67), (68, 69), (70, 71), 72)
OP_SLOTS = (51,)
Q1_SLOT = 6
TIES_G = (8, 104, 144, 176, 232, 240)
TIES_D = (16, 96, 120, 192, 232, 256)
STIES = (-408, -368, -320, -264, 8, 24, 48, 72)

F32 = jnp.float32
BF16 = jnp.bfloat16
NT = (((1,), (1,)), ((), ()))


def _kernel(x_hbm, wq_hbm, wkt_hbm, wvt_hbm, wo_hbm, wg_hbm, wu_hbm, wd_hbm, gw_hbm,
            o_hbm, x_ref, wq_ref, wkv_ref, wod_ref, wgu_ref, gw_ref,
            k4_ref, vt_ref, s0_ref, s1_ref, g_ref, om_ref, acc_ref, out_ref,
            kb_ref, qf_ref, sv_ref, og_ref,
            sem_x, sem_q, sem_o, sem_w, sem_d, sem_m, sem_out):
    S, D = x_ref.shape
    acols = pl.ds(APH * 128, D)
    nkc = S // KC
    nsub = KC // KB
    NQI = H // 4 // GPI
    NIT = (S // TQ) * NQI
    NH = 4 * GPI
    XC = S // NXC
    XH = XC // 2
    FR = TQ // NQI
    NCT = TQ // 128
    RB = KB // NTK
    qscale = (DH ** -0.5) * math.log2(math.e)

    def copy(src, dst, sem):
        return pltpu.make_async_copy(src, dst, sem)

    def start(cps):
        for cp in cps:
            cp.start()

    def wait(cps):
        for cp in cps:
            cp.wait()

    def cp_x(c):
        rows = pl.ds(pl.multiple_of(c * XC, XC), XC)
        return copy(x_hbm.at[rows, :], x_ref.at[rows, :], sem_x.at[c])

    def cp_xh(k, sem):
        rows = pl.ds(k * XH, XH)
        return copy(x_hbm.at[rows, :], x_ref.at[rows, :], sem)

    def cps_q(t):
        return [copy(wq_hbm.at[:, pl.ds((t * GPI + k) * 128, 128)], wq_ref.at[t, k], sem_q.at[t])
                for k in range(GPI)]

    def cp_rows(src, off, r0, nr, sem):
        return copy(src.at[pl.ds(r0, nr), :], wod_ref.at[pl.ds(off + r0, nr), pl.ds(0, D)], sem)

    def cp_wo(t):
        r0 = t * (GPI * 128)
        if not isinstance(t, int):
            r0 = pl.multiple_of(r0, GPI * 128)
        return cp_rows(wo_hbm, 0, r0, GPI * 128, sem_o.at[t])

    def cps_gu(s0, ns, sem):
        cps = []
        for s in range(s0, s0 + ns):
            cols = pl.ds(s * 128, 128)
            cps.append(copy(wg_hbm.at[:, cols], wgu_ref.at[s, 0], sem))
            cps.append(copy(wu_hbm.at[:, cols], wgu_ref.at[s, 1], sem))
        return cps

    def cp_out(b):
        rows = pl.ds(pl.multiple_of(b * FR, FR), FR)
        return copy(out_ref.at[rows, :], o_hbm.at[rows, :], sem_out.at[0])

    def chunk(t):
        return 2 + 13 * (t // 2) + 7 * (t % 2), 7 - t % 2

    def kv_rows(rows, xc):
        kvt = jax.lax.dot_general(wkv_ref[...], xc, NT, preferred_element_type=F32)
        vt_ref[:, rows] = kvt[DH:].astype(BF16)
        kt = kvt[:DH] * qscale
        kk = jnp.concatenate([kt, kt, kt, kt], axis=0).T
        lane = jax.lax.broadcasted_iota(jnp.int32, kk.shape, 1)
        for j in range(4):
            sel = jnp.logical_and(lane >= j * DH, lane < (j + 1) * DH)
            k4_ref[j, rows, :] = jnp.where(sel, kk, 0.0).astype(BF16)

    def gate_rows(rows, xc):
        gw = gw_ref[...].astype(F32).reshape(1, D)
        z = jnp.sum(xc.astype(F32) * gw, axis=-1, keepdims=True)
        g = jnp.broadcast_to(jax.nn.sigmoid(z), (xc.shape[0], 128))
        g_ref[rows, :] = g
        om_ref[rows, :] = 1.0 - g
        return 1.0 - g

    def hidden(xc, om, ks):
        wg0 = jnp.concatenate([wgu_ref[k, 0] for k in ks], axis=1)
        wu0 = jnp.concatenate([wgu_ref[k, 1] for k in ks], axis=1)
        gate = jnp.dot(xc, wg0, preferred_element_type=F32)
        up = jnp.dot(xc, wu0, preferred_element_type=F32)
        om = jnp.concatenate([om] * len(ks), axis=1)
        return (jnp.maximum(gate, 0.0) * up * om).astype(BF16)

    def init_acc(rows, hh):
        w = wod_ref[D:D + hh.shape[1], :D]
        acc_ref[rows, acols] = jnp.dot(hh, w, preferred_element_type=F32)

    def k_table(lo, hi):
        kr = k4_ref[0, lo:hi, :].astype(F32)
        for d in range(DH):
            kb_ref[d, lo:hi, :] = jnp.broadcast_to(kr[:, d:d + 1], (hi - lo, 128))

    small = [copy(wkt_hbm, wkv_ref.at[pl.ds(0, DH), :], sem_m.at[0]),
             copy(wvt_hbm, wkv_ref.at[pl.ds(DH, DH), :], sem_m.at[0]),
             copy(gw_hbm, gw_ref, sem_m.at[0])]
    batch_a = [cp_xh(0, sem_m.at[1])] + cps_gu(0, 1, sem_m.at[1])
    batch_b = [cp_xh(1, sem_m.at[2])] + cps_gu(1, 1, sem_m.at[2])
    cp_wd0 = cp_rows(wd_hbm, D, 0, 256, sem_m.at[0])
    s0, ns = chunk(0)
    gu0 = cps_gu(s0, ns, sem_w.at[0])
    early = [gu0[:3], gu0[3:10], gu0[10:] + cps_q(0),
             [cp_rows(wd_hbm, D, s0 * 128, ns * 128, sem_d.at[0]), cp_wo(0)]]
    start(small)
    start(batch_a)
    wait(small)
    start(batch_b)
    wait(batch_a)

    rows0 = pl.ds(0, XH)
    xc = x_ref[rows0, :]
    om0 = gate_rows(rows0, xc)
    h0 = hidden(xc, om0, [0])
    kv_rows(rows0, xc)

    wait(batch_b)
    cp_wd0.start()
    cp_x(1).start()

    k_table(0, XH)
    h1 = hidden(x_ref[rows0, :], om0, [1])
    rows1 = pl.ds(XH, XH)
    xc = x_ref[rows1, :]
    kv_rows(rows1, xc)
    h2 = hidden(xc, gate_rows(rows1, xc), [0, 1])

    cp_wd0.wait()
    start(early[0])
    k_table(XH, KV)
    init_acc(pl.ds(0, XC), jnp.concatenate([h0, h2[:, :128]], axis=0))
    og_ref[...] = jnp.concatenate([h1, h2[:, 128:]], axis=0)

    def prep(c, carry):
        cp_x(c).wait()

        @pl.when(c + 1 < NXC)
        def _():
            cp_x(c + 1).start()

        for k in range(1, NXC):
            @pl.when(c == k)
            def _():
                start(early[k])

        rows = pl.ds(pl.multiple_of(c * XC, XC), XC)
        xr = x_ref[rows, :]
        kv_rows(rows, xr)
        init_acc(rows, hidden(xr, gate_rows(rows, xr), [0, 1]))
        return carry

    jax.lax.fori_loop(1, NXC, prep, 0)
    for t in range(1, NQI):
        s0, ns = chunk(t)
        start(cps_q(t) + cps_gu(s0, ns, sem_w.at[t])
              + [cp_rows(wd_hbm, D, s0 * 128, ns * 128, sem_d.at[t]), cp_wo(t)])

    def body(n, carry):
        t = jnp.bitwise_and(n, NQI - 1)
        odd = jnp.bitwise_and(n, 1)
        sbase = 2 + 13 * jnp.right_shift(t, 1) + 7 * odd
        sextra = 8 + 13 * jnp.right_shift(t, 1)

        @pl.when(n < NQI)
        def _():
            copy(wq_ref.at[n], wq_ref.at[n], sem_q.at[n]).wait()
            cp_wo(n).wait()

        for par in range(2):
            @pl.when(jnp.logical_and(n < NQI, odd == par))
            def _():
                ns = 7 - par
                blk = wgu_ref.at[pl.ds(sbase, ns)]
                copy(blk, blk, sem_w.at[n]).wait()
                cp_rows(wd_hbm, D, pl.multiple_of(sbase * 128, 128), ns * 128,
                        sem_d.at[n]).wait()

        row0 = pl.multiple_of(jnp.right_shift(n, NQI.bit_length() - 1) * TQ, TQ)
        fb = jnp.where(n >= NQI, n - NQI, n)
        nfin = [0]

        @pl.when(n > NQI)
        def _():
            cp_out(n - NQI - 1).start()

        def finalize_piece():
            k = nfin[0]
            nfin[0] += 1
            if k < FR // 8:
                rows = pl.ds(pl.multiple_of(fb * FR + k * 8, 8), 8)
                out_ref[rows, :] = acc_ref[rows, acols].astype(out_ref.dtype)

        clock = []
        sclock = []
        hist = []
        rot = [0]

        def tick(v, dst=clock):
            dst.append(jnp.minimum(v, -jnp.inf))

        def filler_ticks(res, early=None):
            for ra in (TIES_D if early is None else TIES_G):
                tick(res[ra - 8:ra])
            if early is not None:
                sclock.clear()
                for ra in STIES:
                    tick(res[ra - 8:ra] if ra > 0 else early[ra + 504:ra + 512], sclock)

        def unit(j):
            if j < 12:
                return sbase + j // 2, row0 + (j % 2) * FU
            return sextra, row0 + odd * FU

        hs = {}

        def gate_up(j):
            s, r0 = unit(j)
            rows = pl.ds(pl.multiple_of(r0, FU), FU)
            xh = x_ref[rows, :]
            gate = jnp.dot(xh, wgu_ref[s, 0], preferred_element_type=F32)
            up = jnp.dot(xh, wgu_ref[s, 1], preferred_element_type=F32)
            hh = jnp.maximum(gate, 0.0) * up
            filler_ticks(hh, gate)
            hs[j] = (hh * om_ref[rows, :]).astype(BF16)

        def down(j, half):
            s, r0 = unit(j)
            lo, nr = (0, FU) if half is None else (half * (FU // 2), FU // 2)
            rows = pl.ds(pl.multiple_of(r0 + lo, nr), nr)
            w = wod_ref[pl.ds(pl.multiple_of(D + s * 128, 128), 128), :D]
            res = jnp.dot(hs[j][lo:lo + nr], w, preferred_element_type=F32)
            finalize_piece()
            acc_ref[rows, acols] += res
            if half is None:
                filler_ticks(res[:, D - 128:])
            else:
                for c0 in (0, D - 128):
                    for ra in range(32, nr + 1, 32):
                        tick(res[ra - 8:ra, c0:c0 + 128])

        ogs = {}

        def out_proj(gl):
            rows = pl.ds(row0, TQ)
            w = wod_ref[pl.ds(pl.multiple_of((t * GPI + gl) * 128, 128), 128), :D]
            res = jnp.dot(ogs[gl], w, preferred_element_type=F32)
            finalize_piece()
            acc_ref[rows, acols] += res
            filler_ticks(res[TQ - 256:, D - 128:])

        def out_proj_prev():
            np_ = jnp.maximum(n - 1, 0)
            rp = pl.multiple_of(jnp.right_shift(np_, NQI.bit_length() - 1) * TQ, TQ)
            wrow = jnp.where(n == 0, D + 128, (jnp.bitwise_and(np_, NQI - 1) * GPI + 1) * 128)
            w = wod_ref[pl.ds(pl.multiple_of(wrow, 128), 128), :D]
            acc_ref[pl.ds(rp, TQ), acols] += jnp.dot(og_ref[...], w, preferred_element_type=F32)

        def qproj(gl):
            xt = x_ref[pl.ds(row0, TQ), :]
            q = jnp.dot(xt, wq_ref[t, gl], preferred_element_type=F32)
            qt = q.astype(BF16).T
            qtf = qt.astype(F32)
            for r in range(128):
                qf_ref[gl, r] = jnp.broadcast_to(qtf[r:r + 1, :], (8, TQ))
            return qt

        qg = [qproj(0)]
        out_proj_prev()
        mv = {}

        def vpu_part(j, vp):
            vrows = pl.ds(vp * VR * 8, VR * 8)
            sacc = None
            for d in range(DH):
                kb = kb_ref[d, vrows, :].reshape(VR, 8, 128)
                if len(hist) >= LB:
                    kb = jnp.maximum(kb, hist[-LB][None])
                kb = jnp.concatenate([kb] * NCT, axis=2)
                prod = kb * qf_ref[j // 4, (j % 4) * DH + d][None]
                sacc = prod if sacc is None else sacc + prod
                ix = rot[0] % (VR * NCT)
                rot[0] += 1
                gate_v = jnp.minimum(
                    sacc[ix // NCT, :, (ix % NCT) * 128:(ix % NCT + 1) * 128], -jnp.inf)
                hist.append(gate_v)
            sv_ref[j, vrows, :] = sacc.reshape(VR * 8, TQ)
            for r in range(VR):
                mv[j] = sacc[r] if j not in mv else jnp.maximum(mv[j], sacc[r])
            for cc in range(NCT):
                gate_v = jnp.minimum(mv[j][:, cc * 128:(cc + 1) * 128], gate_v)
            hist[-1] = gate_v

        sched = {}
        for j, slot in enumerate(GU_SLOTS):
            sched.setdefault(slot, []).append((gate_up, (j,)))
        for j, slot in enumerate(DN_SLOTS):
            if isinstance(slot, tuple):
                for half in range(2):
                    sched.setdefault(slot[half], []).append((down, (j, half)))
            else:
                sched.setdefault(slot, []).append((down, (j, None)))
        for gl, slot in enumerate(OP_SLOTS):
            sched.setdefault(slot, []).append((out_proj, (gl,)))

        def fill(slot):
            if slot == Q1_SLOT:
                qg.append(qproj(1))
            for fn, a in sched.get(slot, []):
                fn(*a)
            for j in range(NH):
                if slot == max(j * nkc - 7, 0 if j < 4 else Q1_SLOT):
                    for vp in range(KVS[j] // (8 * VR)):
                        vpu_part(j, vp)

        sbuf = (s0_ref, s1_ref)
        outs = []
        for st in range(NH + 1):
            ja = st if st < NH else None
            jb = st - 1 if st > 0 else None
            m8 = None
            l8 = None
            acc = None
            if jb is not None:
                mu0 = mu_next
            for c in range(nkc):
                base = len(clock)
                fill(st * nkc + c)
                nk = 0
                if ja is not None:
                    base = len(clock)
                    lo_k = max(KVS[ja], c * KC)
                    nk = (c + 1) * KC - lo_k
                if nk > 0:
                    arows = pl.ds(lo_k, nk)
                    s = jnp.dot(k4_ref[ja % 4, arows, :], qg[ja // 4], preferred_element_type=F32)
                    sbuf[ja % 2][arows, :] = s
                    for r in range(nk // 8):
                        sr = s[r * 8:(r + 1) * 8, :]
                        m8 = sr if m8 is None else jnp.maximum(m8, sr)
                        if (r + 1) % (RB // 8) == 0:
                            tc = ((r + 1) // (RB // 8)) % NCT
                            tick(m8[:, tc * 128:(tc + 1) * 128])
                if jb is not None:
                    for tt in range(nsub):
                        k = c * nsub + tt
                        if jb in ONL:
                            nv = -(-KVS[jb] // KB)
                            k = (k + nv) % (nkc * nsub)
                            if k == 0:
                                m2 = jnp.max(jnp.maximum(mu0, mv[jb]), axis=0, keepdims=True)
                                m2 = jnp.broadcast_to(m2, (8, TQ))
                                alpha = jnp.exp2(mu0 - m2)
                                l8 = l8 * alpha
                                acc = acc * alpha[:1]
                                mu0 = m2
                        ps = []
                        for u in range(NTK):
                            lo = k * KB + KB - (u + 1) * RB
                            kv = KVS[jb]
                            if lo + RB <= kv:
                                sv = sv_ref[jb, pl.ds(lo, RB), :]
                            elif lo < kv:
                                sv = jnp.concatenate(
                                    [sv_ref[jb, pl.ds(lo, kv - lo), :],
                                     sbuf[jb % 2][pl.ds(kv, lo + RB - kv), :]], axis=0)
                            else:
                                sv = sbuf[jb % 2][pl.ds(lo, RB), :]
                            gi = tt * NTK + u
                            if ja is not None and c == 0:
                                clk = sclock[gi]
                            else:
                                lag = LAGS[st][c]
                                clk = clock[min(base - lag + gi, len(clock) - 1)]
                            mu = jnp.maximum(mu0, jnp.concatenate([clk] * NCT, axis=1))
                            pu = jnp.exp2(sv.reshape(RB // 8, 8, TQ) - mu[None]).reshape(RB, TQ)
                            for r in reversed(range(RB // 8)):
                                pr = pu[r * 8:(r + 1) * 8, :]
                                l8 = pr if l8 is None else l8 + pr
                            ps.insert(0, pu)
                        p = jnp.concatenate(ps, axis=0).astype(BF16)
                        pv = jnp.dot(vt_ref[:, pl.ds(k * KB, KB)], p,
                                     preferred_element_type=F32)
                        acc = pv if acc is None else acc + pv
                        tick(pv[DH - 8:, :128])
            if jb is not None:
                l = jnp.sum(l8, axis=0, keepdims=True)
                outs.append(acc / l)
                if jb % 4 == 3:
                    og = jnp.concatenate(outs, axis=0).T
                    ogs[jb // 4] = (og * g_ref[pl.ds(row0, TQ), :]).astype(BF16)
                    outs = []
                if jb == NH - 1:
                    fill((NH + 1) * nkc)
                    og_ref[...] = ogs[GPI - 1]
            if ja is not None:
                if ja not in ONL:
                    m8 = jnp.maximum(m8, mv[ja])
                mu_next = jnp.broadcast_to(jnp.max(m8, axis=0, keepdims=True), (8, TQ))
        return carry

    jax.lax.fori_loop(0, NIT, body, 0)

    cp_out(NIT - NQI - 1).start()
    w = wod_ref[D - 128:D, :D]
    for k in range(NQI):
        b = NIT - NQI + k
        rows = pl.ds(b * FR, FR)
        res = jnp.dot(og_ref[k * FR:(k + 1) * FR, :], w, preferred_element_type=F32)
        out_ref[rows, :] = (acc_ref[rows, acols] + res).astype(out_ref.dtype)
        cp_out(b).start()
    copy(out_ref, o_hbm, sem_out.at[0]).wait()


@jax.jit
def pallas_gated_mix__grouped_kv_mqa__glu_gated_reglu__prompt_kernel(
    A_x: jax.Array,
    A_wq: jax.Array,
    A_wk: jax.Array,
    A_wv: jax.Array,
    A_wo: jax.Array,
    B_x: jax.Array,
    B_W_gate: jax.Array,
    B_W_up: jax.Array,
    B_W_down: jax.Array,
    gate_w: jax.Array,
):
    B, S, D = A_x.shape
    F = B_W_gate.shape[1]
    assert (B, S, D, F) == (1, 2048, 1024, 3584)
    x = A_x.reshape(S, D)
    nqi = H // 4 // GPI

    out = pl.pallas_call(
        _kernel,
        in_specs=[pl.BlockSpec(memory_space=pl.ANY)] * 9,
        out_specs=pl.BlockSpec(memory_space=pl.ANY),
        out_shape=jax.ShapeDtypeStruct((S, D), A_x.dtype),
        scratch_shapes=[
            pltpu.VMEM((S, D), BF16),
            pltpu.VMEM((nqi, GPI, D, 128), BF16),
            pltpu.VMEM((2 * DH, D), BF16),
            pltpu.VMEM((D + F, D + PADW), BF16),
            pltpu.VMEM((F // 128, 2, D, 128), BF16),
            pltpu.VMEM((D,), BF16),
            pltpu.VMEM((4, S, 128), BF16),
            pltpu.VMEM((DH, S), BF16),
            pltpu.VMEM((S, TQ), F32),
            pltpu.VMEM((S, TQ), F32),
            pltpu.VMEM((S, 128), F32),
            pltpu.VMEM((S, 128), F32),
            pltpu.VMEM((S, D + 512), F32),
            pltpu.VMEM((S, D), BF16),
            pltpu.VMEM((DH, KV, 128), F32),
            pltpu.VMEM((GPI, 128, 8, TQ), F32),
            pltpu.VMEM((4 * GPI, KV, TQ), F32),
            pltpu.VMEM((TQ, 128), BF16),
            pltpu.SemaphoreType.DMA((NXC,)),
            pltpu.SemaphoreType.DMA((nqi,)),
            pltpu.SemaphoreType.DMA((nqi,)),
            pltpu.SemaphoreType.DMA((nqi,)),
            pltpu.SemaphoreType.DMA((nqi,)),
            pltpu.SemaphoreType.DMA((3,)),
            pltpu.SemaphoreType.DMA((1,)),
        ],
        compiler_params=pltpu.CompilerParams(
            vmem_limit_bytes=110 * 1024 * 1024,
            disable_bounds_checks=True,
            disable_semaphore_checks=True),
        name="gated_mix",
    )(x, A_wq, A_wk.T, A_wv.T, A_wo, B_W_gate, B_W_up, B_W_down, gate_w)
    return out.reshape(B, S, D)
```
